```python
import os as _os
_os.environ.setdefault("JAX_PLATFORMS", "cpu")
import jax
import jax.numpy as jnp

def _softmax(x, axis=-1):
    return jax.nn.softmax(x, axis=axis)
def _gelu(x):
    return jax.nn.gelu(x, approximate=True)
def _silu(x):
    return jax.nn.silu(x)
def _sigmoid(x):
    return jax.nn.sigmoid(x)
def _layernorm(x, axis=-1, eps=1e-5):
    m = jnp.mean(x, axis=axis, keepdims=True)
    v = jnp.var(x, axis=axis, keepdims=True)
    return (x - m) / jnp.sqrt(v + eps)
def _scatter_add(tgt, idx, src, axis=0):
    return tgt.at[idx].add(src)
def _segment_sum(src, seg, n):
    return jax.ops.segment_sum(src, seg, n)
class _Rng:
    def __init__(self, key):
        self._k = key
    def _next(self):
        self._k, sub = jax.random.split(self._k)
        return sub
    def normal(self, shape):
        return jax.random.normal(self._next(), shape, dtype=jnp.bfloat16)
    def randint(self, lo, hi, shape):
        return jax.random.randint(self._next(), shape, lo, hi, dtype=jnp.int32)
    def uniform(self, shape, lo=0.0, hi=1.0):
        return jax.random.uniform(self._next(), shape, jnp.bfloat16, lo, hi)
    def permutation(self, n):
        return jax.random.permutation(self._next(), n)


kernel_name = 'concat_heads__mha_block_cached__mha_block_cached__near_ridge'

def setup_inputs():
    _rng = _Rng(jax.random.key(int.from_bytes(__import__("os").urandom(4), "little")))
    _w = (lambda a: (lambda t: t.astype(jnp.bfloat16) if jnp.issubdtype(t.dtype, jnp.floating) else t)(jnp.asarray(a)))
    def _A_setup():
        B, Sq, D = 8, 144, 640
        H, Sk, Dh = 32, 512, 128
        return {
            "x": _w((lambda *s: _rng.normal(s) * 0.8)(B, Sq, D)),
            "k_cache": _w((lambda *s: _rng.normal(s) * 0.8)(B, H, Sk, Dh)),
            "v_cache": _w((lambda *s: _rng.normal(s) * 0.05)(B, H, Sk, Dh)),
            "wq": _w((lambda *s: _rng.normal(s) * 0.8)(D, H * Dh) * (D ** -0.5)),
            "wo": _w((lambda *s: _rng.normal(s) * 0.05)(H * Dh, D) * ((H * Dh) ** -0.5)),
        }
    _A_in = _A_setup()

    def _B_setup():
        B, Sq, D = 8, 144, 640
        H, Sk, Dh = 32, 512, 128
        return {
            "x": _w((lambda *s: _rng.normal(s) * 0.8)(B, Sq, D)),
            "k_cache": _w((lambda *s: _rng.normal(s) * 0.8)(B, H, Sk, Dh)),
            "v_cache": _w((lambda *s: _rng.normal(s) * 0.05)(B, H, Sk, Dh)),
            "wq": _w((lambda *s: _rng.normal(s) * 0.8)(D, H * Dh) * (D ** -0.5)),
            "wo": _w((lambda *s: _rng.normal(s) * 0.05)(H * Dh, D) * ((H * Dh) ** -0.5)),
        }
    _B_in = _B_setup()

    return {
        "A_x": _A_in["x"],
        "A_k_cache": _A_in["k_cache"],
        "A_v_cache": _A_in["v_cache"],
        "A_wq": _A_in["wq"],
        "A_wo": _A_in["wo"],
        "B_x": _B_in["x"],
        "B_k_cache": _B_in["k_cache"],
        "B_v_cache": _B_in["v_cache"],
        "B_wq": _B_in["wq"],
        "B_wo": _B_in["wo"],
    }

def reference(A_x, A_k_cache, A_v_cache, A_wq, A_wo, B_x, B_k_cache, B_v_cache, B_wq, B_wo):
    def _A_ref(x, k_cache, v_cache, wq, wo):
        B, Sq, D = x.shape
        H, Dh = 32, 128
        q = (lambda x, *d: x.transpose(*d))((x @ wq).reshape(B, Sq, H, Dh), 0, 2, 1, 3)
        scores = jnp.einsum("bhqd,bhkd->bhqk", q, k_cache) * (Dh ** -0.5)
        p = _softmax(scores, axis=-1)
        o = jnp.einsum("bhqk,bhkd->bhqd", p, v_cache)
        return (lambda x, *d: x.transpose(*d))(o, 0, 2, 1, 3).reshape(B, Sq, H * Dh) @ wo

    def _B_ref(x, k_cache, v_cache, wq, wo):
        B, Sq, D = x.shape
        H, Dh = 32, 128
        q = (lambda x, *d: x.transpose(*d))((x @ wq).reshape(B, Sq, H, Dh), 0, 2, 1, 3)
        scores = jnp.einsum("bhqd,bhkd->bhqk", q, k_cache) * (Dh ** -0.5)
        p = _softmax(scores, axis=-1)
        o = jnp.einsum("bhqk,bhkd->bhqd", p, v_cache)
        return (lambda x, *d: x.transpose(*d))(o, 0, 2, 1, 3).reshape(B, Sq, H * Dh) @ wo

    a = _A_ref(A_x, A_k_cache, A_v_cache, A_wq, A_wo)
    b = _B_ref(B_x, B_k_cache, B_v_cache, B_wq, B_wo)
    return jnp.concatenate([a, b], axis=-1)
```

```python
import functools

import jax
import jax.numpy as jnp
from jax import lax
import jax.experimental.pallas as pl
import jax.experimental.pallas.tpu as pltpu


def _recip(l):
    r = pl.reciprocal(l, approx=True)
    return r * (2.0 - l * r)


def _softmax_pv(s, v):
    m = jnp.max(s, axis=-1, keepdims=True)
    p = jnp.exp(s - m)
    l = jnp.sum(p, axis=-1, keepdims=True)
    o = jnp.dot(p.astype(jnp.bfloat16), v, preferred_element_type=jnp.float32)
    return (o * _recip(l)).astype(jnp.bfloat16)


def _qk(q, k):
    return lax.dot_general(q, k, (((1,), (1,)), ((), ())),
                           preferred_element_type=jnp.float32)


def _oproj(acc_ref, outs, wo_ref, nsplit, Sq):
    nb = len(outs) // nsplit
    for c in range(nsplit):
        o = jnp.concatenate(outs[c * nb:(c + 1) * nb], axis=0) if nb > 1 else outs[c]
        r0 = c * nb * Sq
        acc_ref[r0:r0 + nb * Sq, :] += jnp.dot(
            o, wo_ref[...], preferred_element_type=jnp.float32)


def _kernel(xa_ref, ka_ref, va_ref, wqa_ref, woa_ref,
            xb_ref, kb_ref, vb_ref, wqb_ref, wob_ref,
            o_ref, acca_ref, accb_ref, *, B, Sq, D, scale):
    h = pl.program_id(0)

    @pl.when(h == 0)
    def _():
        acca_ref[...] = jnp.zeros_like(acca_ref)
        accb_ref[...] = jnp.zeros_like(accb_ref)

    qa = (jnp.dot(xa_ref[...], wqa_ref[...], preferred_element_type=jnp.float32)
          * scale).astype(jnp.bfloat16)
    qb = (jnp.dot(xb_ref[...], wqb_ref[...], preferred_element_type=jnp.float32)
          * scale).astype(jnp.bfloat16)

    items = ([(qa, ka_ref, va_ref, b) for b in range(B)]
             + [(qb, kb_ref, vb_ref, b) for b in range(B)])
    outs = []
    q, k_ref, _, b = items[0]
    s_next = _qk(q[b * Sq:(b + 1) * Sq, :], k_ref[b])
    for i in range(len(items)):
        s = s_next
        if i + 1 < len(items):
            q, k_ref, _, b = items[i + 1]
            s_next = _qk(q[b * Sq:(b + 1) * Sq, :], k_ref[b])
        _, _, v_ref, b = items[i]
        outs.append(_softmax_pv(s, v_ref[b]))
        if i == B - 1:
            _oproj(acca_ref, outs[:B], woa_ref, 1, Sq)
    _oproj(accb_ref, outs[B:], wob_ref, 4, Sq)

    @pl.when(h == pl.num_programs(0) - 1)
    def _():
        o_ref[:, 0:D] = acca_ref[...].astype(o_ref.dtype)
        o_ref[:, D:2 * D] = accb_ref[...].astype(o_ref.dtype)


@jax.jit
def pallas_concat_heads__mha_block_cached__mha_block_cached__near_ridge_kernel(
    A_x: jax.Array,
    A_k_cache: jax.Array,
    A_v_cache: jax.Array,
    A_wq: jax.Array,
    A_wo: jax.Array,
    B_x: jax.Array,
    B_k_cache: jax.Array,
    B_v_cache: jax.Array,
    B_wq: jax.Array,
    B_wo: jax.Array,
):
    B, Sq, D = A_x.shape
    _, H, Sk, Dh = A_k_cache.shape
    M = B * Sq
    scale = float(Dh) ** -0.5

    xa = A_x.reshape(M, D)
    xb = B_x.reshape(M, D)

    x_spec = pl.BlockSpec((M, D), lambda h: (0, 0))
    kv_spec = pl.BlockSpec((B, None, Sk, Dh), lambda h: (0, h, 0, 0))
    wq_spec = pl.BlockSpec((D, Dh), lambda h: (0, h))
    wo_spec = pl.BlockSpec((Dh, D), lambda h: (h, 0))

    out = pl.pallas_call(
        functools.partial(_kernel, B=B, Sq=Sq, D=D, scale=scale),
        grid=(H,),
        in_specs=[x_spec, kv_spec, kv_spec, wq_spec, wo_spec] * 2,
        out_specs=pl.BlockSpec((M, 2 * D), lambda h: (0, 0)),
        out_shape=jax.ShapeDtypeStruct((M, 2 * D), A_x.dtype),
        scratch_shapes=[
            pltpu.VMEM((M, D), jnp.float32),
            pltpu.VMEM((M, D), jnp.float32),
        ],
        compiler_params=pltpu.CompilerParams(
            dimension_semantics=("arbitrary",),
            vmem_limit_bytes=64 * 1024 * 1024,
        ),
    )(xa, A_k_cache, A_v_cache, A_wq, A_wo, xb, B_k_cache, B_v_cache, B_wq, B_wo)
    return out.reshape(B, Sq, 2 * D)
```
